```python
import os as _os
_os.environ.setdefault("JAX_PLATFORMS", "cpu")
import jax
import jax.numpy as jnp

def _softmax(x, axis=-1):
    return jax.nn.softmax(x, axis=axis)
def _gelu(x):
    return jax.nn.gelu(x, approximate=True)
def _silu(x):
    return jax.nn.silu(x)
def _sigmoid(x):
    return jax.nn.sigmoid(x)
def _layernorm(x, axis=-1, eps=1e-5):
    m = jnp.mean(x, axis=axis, keepdims=True)
    v = jnp.var(x, axis=axis, keepdims=True)
    return (x - m) / jnp.sqrt(v + eps)
def _scatter_add(tgt, idx, src, axis=0):
    return tgt.at[idx].add(src)
def _segment_sum(src, seg, n):
    return jax.ops.segment_sum(src, seg, n)
class _Rng:
    def __init__(self, key):
        self._k = key
    def _next(self):
        self._k, sub = jax.random.split(self._k)
        return sub
    def normal(self, shape):
        return jax.random.normal(self._next(), shape, dtype=jnp.bfloat16)
    def randint(self, lo, hi, shape):
        return jax.random.randint(self._next(), shape, lo, hi, dtype=jnp.int32)
    def uniform(self, shape, lo=0.0, hi=1.0):
        return jax.random.uniform(self._next(), shape, jnp.bfloat16, lo, hi)
    def permutation(self, n):
        return jax.random.permutation(self._next(), n)


kernel_name = 'concat_heads__mha_block_cached__gqa_block_cached__decode'

def setup_inputs():
    _rng = _Rng(jax.random.key(int.from_bytes(__import__("os").urandom(4), "little")))
    _w = (lambda a: (lambda t: t.astype(jnp.bfloat16) if jnp.issubdtype(t.dtype, jnp.floating) else t)(jnp.asarray(a)))
    def _A_setup():
        B, Sq, D = 1, 1, 512
        H, Sk, Dh = 32, 4096, 128
        return {
            "x": _w((lambda *s: _rng.normal(s) * 0.8)(B, Sq, D)),
            "k_cache": _w((lambda *s: _rng.normal(s) * 0.8)(B, H, Sk, Dh)),
            "v_cache": _w((lambda *s: _rng.normal(s) * 0.05)(B, H, Sk, Dh)),
            "wq": _w((lambda *s: _rng.normal(s) * 0.8)(D, H * Dh) * (D ** -0.5)),
            "wo": _w((lambda *s: _rng.normal(s) * 0.05)(H * Dh, D) * ((H * Dh) ** -0.5)),
        }
    _A_in = _A_setup()

    def _B_setup():
        B, Sq, D = 1, 1, 512
        Hq, Hkv, Sk, Dh = 32, 32, 4096, 128
        assert Hq % Hkv == 0, (Hq, Hkv)
        return {
            "x": _w((lambda *s: _rng.normal(s) * 0.8)(B, Sq, D)),
            "k_cache": _w((lambda *s: _rng.normal(s) * 0.8)(B, Hkv, Sk, Dh)),
            "v_cache": _w((lambda *s: _rng.normal(s) * 0.05)(B, Hkv, Sk, Dh)),
            "wq": _w((lambda *s: _rng.normal(s) * 0.8)(D, Hq * Dh) * (D ** -0.5)),
            "wo": _w((lambda *s: _rng.normal(s) * 0.05)(Hq * Dh, D) * ((Hq * Dh) ** -0.5)),
        }
    _B_in = _B_setup()

    return {
        "A_x": _A_in["x"],
        "A_k_cache": _A_in["k_cache"],
        "A_v_cache": _A_in["v_cache"],
        "A_wq": _A_in["wq"],
        "A_wo": _A_in["wo"],
        "B_x": _B_in["x"],
        "B_k_cache": _B_in["k_cache"],
        "B_v_cache": _B_in["v_cache"],
        "B_wq": _B_in["wq"],
        "B_wo": _B_in["wo"],
    }

def reference(A_x, A_k_cache, A_v_cache, A_wq, A_wo, B_x, B_k_cache, B_v_cache, B_wq, B_wo):
    def _A_ref(x, k_cache, v_cache, wq, wo):
        B, Sq, D = x.shape
        H, Dh = 32, 128
        q = (lambda x, *d: x.transpose(*d))((x @ wq).reshape(B, Sq, H, Dh), 0, 2, 1, 3)
        scores = jnp.einsum("bhqd,bhkd->bhqk", q, k_cache) * (Dh ** -0.5)
        p = _softmax(scores, axis=-1)
        o = jnp.einsum("bhqk,bhkd->bhqd", p, v_cache)
        return (lambda x, *d: x.transpose(*d))(o, 0, 2, 1, 3).reshape(B, Sq, H * Dh) @ wo

    def _B_ref(x, k_cache, v_cache, wq, wo):
        B, Sq, D = x.shape
        Hq, Dh = 32, 128
        Hkv = k_cache.shape[1]
        rep = Hq // Hkv
        q = (lambda x, *d: x.transpose(*d))((x @ wq).reshape(B, Sq, Hq, Dh), 0, 2, 1, 3)
        k = jnp.repeat(k_cache, rep, axis=1)
        v = jnp.repeat(v_cache, rep, axis=1)
        scores = jnp.einsum("bhqd,bhkd->bhqk", q, k) * (Dh ** -0.5)
        p = _softmax(scores, axis=-1)
        o = jnp.einsum("bhqk,bhkd->bhqd", p, v)
        return (lambda x, *d: x.transpose(*d))(o, 0, 2, 1, 3).reshape(B, Sq, Hq * Dh) @ wo

    a = _A_ref(A_x, A_k_cache, A_v_cache, A_wq, A_wo)
    b = _B_ref(B_x, B_k_cache, B_v_cache, B_wq, B_wo)
    return jnp.concatenate([a, b], axis=-1)
```

```python
import jax
import jax.numpy as jnp
from jax import lax
import jax.experimental.pallas as pl
import jax.experimental.pallas.tpu as pltpu

H, SK, DH, D = 32, 4096, 128, 512
HD = H * DH
SCALE = DH ** -0.5
CH = 128
HALF = SK // 2
NPIECE = 4


def _kernel(ax, ak, av, awq, awo, bx, bk, bv, bwq, bwo, out,
            kbuf, vbuf, wqbuf, wobuf, xbuf, qbuf, pbuf, lbuf, acc,
            ksem, vsem, wsem, xsem, tsem):
    ks, vs = (ak, bk), (av, bv)
    wqs, wos, xs = (awq, bwq), (awo, bwo), (ax, bx)

    def kcopy(ab, h, slot, r0):
        return pltpu.make_async_copy(ks[ab].at[0, h, pl.ds(r0, CH), :],
                                     kbuf.at[slot, ab, pl.ds(r0, CH), :],
                                     ksem.at[slot, ab])

    def vcopy(ab, h, slot, r0, sem=None):
        return pltpu.make_async_copy(vs[ab].at[0, h, pl.ds(r0, CH), :],
                                     vbuf.at[slot, ab, pl.ds(r0, CH), :],
                                     vsem.at[slot, ab] if sem is None else sem)

    def issue_kv(h, slot, i0, n):
        def body(i, c):
            for s in range(2):
                r0 = pl.multiple_of(s * HALF + i * CH, CH)
                for ab in range(2):
                    kcopy(ab, h, slot, r0).start(priority=0)
                    vcopy(ab, h, slot, r0).start(priority=1)
            return c
        lax.fori_loop(i0, i0 + n, body, 0)

    def wait_all(buf, sem):
        pltpu.make_async_copy(buf, buf, sem).wait()

    for ab in range(2):
        pltpu.make_async_copy(xs[ab], xbuf.at[ab], xsem.at[ab]).start(priority=0)

    def wbody(i, c):
        for s in range(2):
            j = s * 64 + i
            qr = pl.multiple_of((j // 2) * 8, 8)
            qc = pl.multiple_of((j % 2) * 2048, 2048)
            orow = pl.multiple_of(j * 32, 32)
            for ab in range(2):
                pltpu.make_async_copy(wqs[ab].at[pl.ds(qr, 8), pl.ds(qc, 2048)],
                                      wqbuf.at[ab, pl.ds(qr, 8), pl.ds(qc, 2048)],
                                      wsem.at[0, ab]).start(priority=0)
                pltpu.make_async_copy(wos[ab].at[pl.ds(orow, 32), :],
                                      wobuf.at[ab, pl.ds(orow, 32), :],
                                      wsem.at[1, ab]).start(priority=1)
        return c
    lax.fori_loop(0, 64, wbody, 0)

    def compute_q(ab):
        pltpu.make_async_copy(xs[ab], xbuf.at[ab], xsem.at[ab]).wait()
        wait_all(wqbuf.at[ab], wsem.at[0, ab])
        x = jnp.broadcast_to(xbuf[ab, 0], (8, D))
        q = jnp.dot(x, wqbuf[ab], preferred_element_type=jnp.float32)
        for h in range(H):
            qbuf[ab, h] = q[:, h * DH:(h + 1) * DH]

    issue_kv(0, 0, 0, 8)
    compute_q(0)
    issue_kv(0, 0, 8, 8)
    compute_q(1)
    for ab in range(2):
        wait_all(wobuf.at[ab], wsem.at[1, ab])
    acc[...] = jnp.zeros_like(acc)

    def scores(ab, h, slot):
        q = qbuf[ab, h].astype(jnp.bfloat16)
        s = lax.dot_general(q, kbuf[slot, ab], (((1,), (1,)), ((), ())),
                            preferred_element_type=jnp.float32) * SCALE
        m = jnp.max(s, axis=-1, keepdims=True)
        p = jnp.exp(s - m)
        l = jnp.sum(p, axis=-1, keepdims=True)
        pbuf[ab] = p.astype(jnp.bfloat16)
        lbuf[ab] = jnp.broadcast_to(l, (8, DH))

    def proj(ab, h, o):
        o = (o / lbuf[ab]).astype(jnp.bfloat16)
        r0 = pl.multiple_of(h * DH, DH)
        return jnp.dot(o, wobuf[ab, pl.ds(r0, DH), :],
                       preferred_element_type=jnp.float32)

    def pv(ab, h, slot):
        o = jnp.dot(pbuf[ab], vbuf[slot, ab], preferred_element_type=jnp.float32)
        acc[ab] += proj(ab, h, o)

    def step(h, issue1, issue2):
        slot = h % 2
        issue1()
        for ab in range(2):
            wait_all(kbuf.at[slot, ab], ksem.at[slot, ab])
        for ab in range(2):
            scores(ab, h, slot)
        issue2()
        for ab in range(2):
            wait_all(vbuf.at[slot, ab], vsem.at[slot, ab])
        for ab in range(2):
            pv(ab, h, slot)

    def body(h, c):
        nslot = (h + 1) % 2
        step(h, lambda: issue_kv(h + 1, nslot, 0, 8),
             lambda: issue_kv(h + 1, nslot, 8, 8))
        return c

    lax.fori_loop(0, H - 2, body, 0)

    hl = H - 1
    sl = hl % 2
    pr = SK // NPIECE

    def issue_last_k():
        def b(i, c):
            for s in range(2):
                r0 = pl.multiple_of(s * HALF + i * CH, CH)
                kcopy(0, hl, sl, r0).start(priority=0)
                kcopy(1, hl, sl, r0).start(priority=1)
            return c
        lax.fori_loop(0, HALF // CH, b, 0)

    def issue_last_v():
        for pc in range(NPIECE):
            def b(i, c, pc=pc):
                r0 = pl.multiple_of(pc * pr + i * CH, CH)
                vcopy(0, hl, sl, r0).start(priority=0)
                vcopy(1, hl, sl, r0, tsem.at[pc]).start(priority=1)
                return c
            lax.fori_loop(0, pr // CH, b, 0)

    step(H - 2, issue_last_k, issue_last_v)
    wait_all(kbuf.at[sl, 0], ksem.at[sl, 0])
    scores(0, hl, sl)
    wait_all(kbuf.at[sl, 1], ksem.at[sl, 1])
    scores(1, hl, sl)
    wait_all(vbuf.at[sl, 0], vsem.at[sl, 0])
    pv(0, hl, sl)
    o = jnp.zeros((8, DH), jnp.float32)
    for pc in range(NPIECE):
        piece = vbuf.at[sl, 1, pl.ds(pc * pr, pr), :]
        wait_all(piece, tsem.at[pc])
        o = o + jnp.dot(pbuf[1, :, pl.ds(pc * pr, pr)], piece[...],
                        preferred_element_type=jnp.float32)
    ob = acc[1] + proj(1, hl, o)
    out[0] = jnp.concatenate([acc[0, 0:1, :], ob[0:1, :]], axis=-1).astype(out.dtype)


@jax.jit
def pallas_concat_heads__mha_block_cached__gqa_block_cached__decode_kernel(
    A_x: jax.Array,
    A_k_cache: jax.Array,
    A_v_cache: jax.Array,
    A_wq: jax.Array,
    A_wo: jax.Array,
    B_x: jax.Array,
    B_k_cache: jax.Array,
    B_v_cache: jax.Array,
    B_wq: jax.Array,
    B_wo: jax.Array,
):
    bf = jnp.bfloat16
    return pl.pallas_call(
        _kernel,
        in_specs=[pl.BlockSpec(memory_space=pl.ANY)] * 10,
        out_specs=pl.BlockSpec(memory_space=pltpu.VMEM),
        out_shape=jax.ShapeDtypeStruct((1, 1, 2 * D), bf),
        scratch_shapes=[
            pltpu.VMEM((2, 2, SK, DH), bf),
            pltpu.VMEM((2, 2, SK, DH), bf),
            pltpu.VMEM((2, D, HD), bf),
            pltpu.VMEM((2, HD, D), bf),
            pltpu.VMEM((2, 1, 1, D), bf),
            pltpu.VMEM((2, H, 8, DH), jnp.float32),
            pltpu.VMEM((2, 8, SK), bf),
            pltpu.VMEM((2, 8, DH), jnp.float32),
            pltpu.VMEM((2, 8, D), jnp.float32),
            pltpu.SemaphoreType.DMA((2, 2)),
            pltpu.SemaphoreType.DMA((2, 2)),
            pltpu.SemaphoreType.DMA((2, 2)),
            pltpu.SemaphoreType.DMA((2,)),
            pltpu.SemaphoreType.DMA((NPIECE,)),
        ],
        compiler_params=pltpu.CompilerParams(vmem_limit_bytes=64 * 1024 * 1024),
    )(A_x, A_k_cache, A_v_cache, A_wq, A_wo, B_x, B_k_cache, B_v_cache, B_wq, B_wo)
```

```python
import jax
import jax.numpy as jnp
from jax import lax
import jax.experimental.pallas as pl
import jax.experimental.pallas.tpu as pltpu

H, SK, DH, D = 32, 4096, 128, 512
HD = H * DH
SCALE = DH ** -0.5
NSL = 3
LEAD = 3
OFF = (112, 120)
TINY = 8

SEM_K, SEM_V, SEM_Q, SEM_X, SEM_O = 0, NSL, 2 * NSL, 2 * NSL + 1, 2 * NSL + 2

_GROUP_LIST = (
    [(ab, h) for ab in range(2) for h in (0, 1, 2, 3, 12, 13, 14, 15)],
    [(ab, h) for ab in range(2) for h in (4, 5, 6, 7, 16, 17, 18, 19)],
    [(ab, h) for ab in range(2) for h in (8, 20, 24, 28)],
    [(ab, h) for ab in range(2) for h in (9, 21, 25, 29)],
    [(ab, h) for ab in range(2) for h in (10, 22, 26, 30)],
    [(0, 27), (0, 11), (1, 27)],
    [(1, 11), (0, 23), (1, 23)],
    [(0, 31), (1, 31)],
)
_GROUP_OF = {key: g for g, keys in enumerate(_GROUP_LIST) for key in keys}
NSEM = SEM_O + len(_GROUP_LIST)


def _stream(k):
    return k % 2, (k // 2) % 2, k // 4


def _kernel(ax, ak, av, awq, awo, bx, bk, bv, bwq, bwo, out,
            kbuf, vbuf, wqbuf, wobuf, xbuf, qbuf, pbuf, lbuf, obuf, sems):
    kv_hbm = ((ak, bk), (av, bv))
    kv_buf = (kbuf, vbuf)
    kv_sem = (SEM_K, SEM_V)
    wqs, wos, xs = (awq, bwq), (awo, bwo), (ax, bx)

    def al(v):
        return v if isinstance(v, int) else pl.multiple_of(v, 8)

    def head(h):
        return (h, h % NSL)

    def wait_all(buf, sem):
        pltpu.make_async_copy(buf, buf, sems.at[sem]).wait()

    def loop(lo, hi, f):
        lax.fori_loop(lo, hi, lambda i, c: (f(i), c)[1], 0)

    def kv_cp(kv, ab, hs, r0, n, prio):
        h, slot = hs
        pltpu.make_async_copy(kv_hbm[kv][ab].at[0, h, pl.ds(r0, n), :],
                              kv_buf[kv].at[slot, ab, pl.ds(r0, n), :],
                              sems.at[kv_sem[kv] + slot]).start(priority=prio)

    def kv_first(kv, ab, s, hs, i, split):
        r0 = al(OFF[ab] + 256 * (8 * s + i))
        if split:
            kv_cp(kv, ab, hs, r0, 64, 1)
            kv_cp(kv, ab, hs, al(r0 + 64), 64, 1)
        else:
            kv_cp(kv, ab, hs, r0, 128, 1)

    def kv_second(kv, ab, s, hs, i, last, nxt):
        if last and s == 1:
            kv_cp(kv, ab, hs, SK - 128 + OFF[ab], 128 - OFF[ab], 0)
            if nxt is not None:
                kv_cp(kv, ab, nxt, 0, OFF[ab], 0)
        else:
            kv_cp(kv, ab, hs, al(OFF[ab] + 128 + 256 * (8 * s + i)), 128, 0)

    def wq_cp(ab, rb, c0, n, prio):
        r = al(rb * 8)
        pltpu.make_async_copy(wqs[ab].at[pl.ds(r, 8), pl.ds(c0, n)],
                              wqbuf.at[ab, pl.ds(r, 8), pl.ds(c0, n)],
                              sems.at[SEM_Q]).start(priority=prio)

    def wq_first(k, i):
        ab, s = k % 2, k // 2
        c0 = OFF[ab] * 16
        if k == 0:
            wq_cp(ab, 16 * s + i, c0, 1024, 1)
            wq_cp(ab, 16 * s + i, c0 + 1024, 1024, 1)
        else:
            wq_cp(ab, 16 * s + i, c0, 2048, 1)

    def wq_second(k, i):
        ab, s = k % 2, k // 2
        c0 = OFF[ab] * 16
        wq_cp(ab, 16 * s + i, c0 + 2048, 2048 - c0, 0)
        wq_cp(ab, (16 * s + i + 1) & 63, 0, c0, 0)

    issued = [0] * len(_GROUP_LIST)

    def wo_rect(ab, r0, n, c0, nc, prio):
        g = _GROUP_OF[(ab, r0 // DH)]
        assert (r0 + n - 1) // DH == r0 // DH
        issued[g] += n * nc
        pltpu.make_async_copy(wos[ab].at[pl.ds(r0, n), pl.ds(c0, nc)],
                              wobuf.at[ab, pl.ds(r0, n), pl.ds(c0, nc)],
                              sems.at[SEM_O + g]).start(priority=prio)

    def wo_tiles(ab, t0, t1, prio):
        if t0 % 4:
            e = min(t1, (t0 // 4 + 1) * 4)
            wo_rect(ab, (t0 // 4) * 8, 8, (t0 % 4) * 128, (e - t0) * 128, prio)
            t0 = e
        if t1 // 4 > t0 // 4:
            wo_rect(ab, (t0 // 4) * 8, (t1 // 4 - t0 // 4) * 8, 0, D, prio)
            t0 = (t1 // 4) * 4
        if t1 > t0:
            wo_rect(ab, (t0 // 4) * 8, 8, 0, (t1 - t0) * 128, prio)

    def compute_q(ab):
        x = jnp.broadcast_to(xbuf[ab, 0], (8, D))
        q = jnp.dot(x, wqbuf[ab], preferred_element_type=jnp.float32)
        for h in range(H):
            qbuf[ab, h] = q[:, h * DH:(h + 1) * DH]

    def scores(hs):
        h, slot = hs
        wait_all(kbuf.at[slot], SEM_K + slot)
        for ab in range(2):
            q = qbuf[ab, h].astype(jnp.bfloat16)
            s = lax.dot_general(q, kbuf[slot, ab], (((1,), (1,)), ((), ())),
                                preferred_element_type=jnp.float32) * SCALE
            m = jnp.max(s, axis=-1, keepdims=True)
            p = jnp.exp(s - m)
            l = jnp.sum(p, axis=-1, keepdims=True)
            pbuf[ab] = p.astype(jnp.bfloat16)
            lbuf[ab] = jnp.broadcast_to(1.0 / l, (8, DH))

    def pv(hs):
        h, slot = hs
        wait_all(vbuf.at[slot], SEM_V + slot)
        for ab in range(2):
            o = jnp.dot(pbuf[ab], vbuf[slot, ab], preferred_element_type=jnp.float32)
            obuf[ab, h] = o * lbuf[ab]

    acc = [jnp.zeros((8, D), jnp.float32)] * 2

    def proj(g):
        assert issued[g] == len(_GROUP_LIST[g]) * DH * D
        for ab, h in _GROUP_LIST[g]:
            wait_all(wobuf.at[ab, pl.ds(h * DH, DH), :], SEM_O + g)
        for ab, h in _GROUP_LIST[g]:
            acc[ab] = acc[ab] + jnp.dot(obuf[ab, h].astype(jnp.bfloat16),
                                        wobuf[ab, h * DH:(h + 1) * DH, :],
                                        preferred_element_type=jnp.float32)

    for ab in range(2):
        pltpu.make_async_copy(xs[ab], xbuf.at[ab], sems.at[SEM_X]).start(priority=0)
    for i in range(LEAD):
        for k in range(8):
            wq_first(k, i)

    def w_round(i):
        for k in range(8):
            wq_second(k, i)
            wq_first(k, i + LEAD)

    def w_round_last(i):
        for k in range(8):
            wq_second(k, i)
            kv_first(*_stream(k), head(0), i - (16 - LEAD), k == 0)

    loop(0, 16 - LEAD, w_round)
    loop(16 - LEAD, 16, w_round_last)
    for kv in range(2):
        for ab in range(2):
            kv_cp(kv, ab, head(0), 0, OFF[ab], 0)

    def kv_round(cur, nxt, i, same, last):
        for k in range(8):
            kv, ab, s = _stream(k)
            kv_second(kv, ab, s, cur, i, last, nxt)
            if same:
                kv_first(kv, ab, s, cur, i + LEAD, k == 0)
            else:
                kv_first(kv, ab, s, nxt, i + LEAD - 8, k == 0)

    def body(b, slots):
        sp, sc, sn = slots
        prev, cur, nxt = (b - 1, sp), (b, sc), (b + 1, sn)
        loop(0, 8 - LEAD, lambda i: kv_round(cur, nxt, i, True, False))

        @pl.when(b == 0)
        def _():
            wait_all(xbuf, SEM_X)
            wait_all(wqbuf, SEM_Q)
            compute_q(0)

        @pl.when(b > 0)
        def _():
            scores(prev)

        loop(8 - LEAD, 7, lambda i: kv_round(cur, nxt, i, False, False))
        kv_round(cur, nxt, 7, False, True)

        @pl.when(b == 0)
        def _():
            compute_q(1)

        @pl.when(b > 0)
        def _():
            pv(prev)

        return sc, sn, sp

    lax.fori_loop(0, H - 2, body, (jnp.int32(2), jnp.int32(0), jnp.int32(1)))

    p0, p1 = {}, {}

    def at(b, i, k=0):
        return 64 * b + 8 * i + k

    def add_kv(b, k, kv, h, nxt):
        _, ab, s = _stream(k)
        for i in range(8):
            p0[at(b, i, k)] = (lambda i=i: kv_second(kv, ab, s, head(h), i, i == 7, nxt))
            p1[at(b, i, k)] = (lambda i=i: kv_first(kv, ab, s, head(h), i, k == 0))

    def add_wo(b, k, r0, rounds):
        ab = _stream(k)[1]
        o = OFF[ab] // 8
        tb, te = r0 // 2, (r0 + 64 * rounds) // 2
        for i in range(rounds + 1):
            lo, hi = max(tb, tb + 32 * (i - 1) + o), min(te, tb + 32 * i + o)
            m0, m1 = (tb, tb + 8) if i == 0 else (tb + 32 * i - 16, tb + 32 * i)

            def f0(lo=lo, hi=hi, m0=m0, m1=m1):
                wo_tiles(ab, lo, m0, 0)
                wo_tiles(ab, m1, hi, 0)

            def f1(m0=m0, m1=m1):
                if k == 0:
                    wo_tiles(ab, m0, (m0 + m1) // 2, 1)
                    wo_tiles(ab, (m0 + m1) // 2, m1, 1)
                else:
                    wo_tiles(ab, m0, m1, 1)

            p0[at(b, i, k)] = f0
            p1[at(b, i, k)] = f1

    for k in range(8):
        kv, _, s = _stream(k)
        add_kv(30, k, kv, 30, head(31))
        if kv == 0:
            add_kv(31, k, 0, 31, None)
            add_kv(32, k, 1, 31, None)
            add_wo(33, k, 3072 + 512 * s, 8 if s == 0 else 6)
        else:
            add_wo(31, k, 1536 * s, 24)
    tiny = [(ab, 31 * DH + r) for ab in range(2) for r in range(0, DH, TINY)]
    t_end = max(p0) + 1
    for t in range(max(p1) + 1, t_end + 8 * LEAD):
        if t - 8 * LEAD in p0:
            ab, r = tiny.pop(0)
            p1[t] = (lambda ab=ab, r=r: wo_rect(ab, r, TINY, 0, D, 1))

    pos = [at(30, 0)]

    def issue(upto):
        for t in range(pos[0], upto):
            if t in p0:
                p0[t]()
            if t + 8 * LEAD in p1:
                p1[t + 8 * LEAD]()
        pos[0] = upto

    issue(at(30, 5)); scores(head(29))
    issue(at(31, 0)); pv(head(29))
    issue(at(31, 5)); scores(head(30))
    issue(at(32, 0)); pv(head(30))
    issue(at(32, 5)); scores(head(31))
    issue(at(33, 0)); proj(0)
    issue(at(33, 3)); pv(head(31))
    issue(at(33, 4)); proj(1)
    issue(at(33, 6)); proj(2)
    issue(at(33, 8)); proj(3)
    issue(t_end)
    for ab, r in tiny:
        wo_rect(ab, r, TINY, 0, D, 1)
    for g in range(4, len(_GROUP_LIST)):
        proj(g)
    out[0] = jnp.concatenate([acc[0][0:1, :], acc[1][0:1, :]], axis=-1).astype(out.dtype)


@jax.jit
def pallas_concat_heads__mha_block_cached__gqa_block_cached__decode_kernel(
    A_x: jax.Array,
    A_k_cache: jax.Array,
    A_v_cache: jax.Array,
    A_wq: jax.Array,
    A_wo: jax.Array,
    B_x: jax.Array,
    B_k_cache: jax.Array,
    B_v_cache: jax.Array,
    B_wq: jax.Array,
    B_wo: jax.Array,
):
    bf = jnp.bfloat16
    return pl.pallas_call(
        _kernel,
        in_specs=[pl.BlockSpec(memory_space=pl.ANY)] * 10,
        out_specs=pl.BlockSpec(memory_space=pltpu.VMEM),
        out_shape=jax.ShapeDtypeStruct((1, 1, 2 * D), bf),
        scratch_shapes=[
            pltpu.VMEM((NSL, 2, SK, DH), bf),
            pltpu.VMEM((NSL, 2, SK, DH), bf),
            pltpu.VMEM((2, D, HD), bf),
            pltpu.VMEM((2, HD, D), bf),
            pltpu.VMEM((2, 1, 1, D), bf),
            pltpu.VMEM((2, H, 8, DH), jnp.float32),
            pltpu.VMEM((2, 8, SK), bf),
            pltpu.VMEM((2, 8, DH), jnp.float32),
            pltpu.VMEM((2, H, 8, DH), jnp.float32),
            pltpu.SemaphoreType.DMA((NSEM,)),
        ],
        compiler_params=pltpu.CompilerParams(
            vmem_limit_bytes=64 * 1024 * 1024,
            disable_semaphore_checks=True,
        ),
    )(A_x, A_k_cache, A_v_cache, A_wq, A_wo, B_x, B_k_cache, B_v_cache, B_wq, B_wo)
```

```python
import jax
import jax.numpy as jnp
from jax import lax
import jax.experimental.pallas as pl
import jax.experimental.pallas.tpu as pltpu

H, SK, DH, D = 32, 4096, 128, 512
HD = H * DH
SCALE = DH ** -0.5
NSL = 3
LEAD = 3
OFF = (112, 120)
TINY = 8
VP = ((0, 0, 128), (1, 0, 96), (1, 96, 128))

SEM_K, SEM_V, SEM_Q, SEM_X, SEM_O = 0, NSL, 2 * NSL, 2 * NSL + 1, 2 * NSL + 2

_GROUP_LIST = (
    [(ab, h) for ab in range(2) for h in (0, 1, 2, 3, 12, 13, 14, 15)],
    [(ab, h) for ab in range(2) for h in (4, 5, 6, 7, 16, 17, 18, 19)],
    [(ab, h) for ab in range(2) for h in (8, 20, 24, 28)],
    [(ab, h) for ab in range(2) for h in (9, 21, 25, 29)],
    [(ab, h) for ab in range(2) for h in (10, 22, 26, 30)],
    [(0, 27), (0, 11), (1, 27)],
    [(1, 11), (0, 23), (1, 23)],
)
_GROUP_OF = {key: g for g, keys in enumerate(_GROUP_LIST) for key in keys}
SEM_T = SEM_O + len(_GROUP_LIST)
NSEM = SEM_T + len(VP)


def _stream(k):
    return k % 2, (k // 2) % 2, k // 4


def _kernel(ax, ak, av, awq, awo, bx, bk, bv, bwq, bwo, out,
            kbuf, vbuf, wqbuf, wobuf, xbuf, qbuf, pbuf, lbuf, obuf, tbuf, sems):
    kv_hbm = ((ak, bk), (av, bv))
    kv_buf = (kbuf, vbuf)
    kv_sem = (SEM_K, SEM_V)
    wqs, wos, xs = (awq, bwq), (awo, bwo), (ax, bx)

    def al(v):
        return v if isinstance(v, int) else pl.multiple_of(v, 8)

    def head(h):
        return (h, h % NSL)

    def wait_all(buf, sem):
        pltpu.make_async_copy(buf, buf, sems.at[sem]).wait()

    def loop(lo, hi, f):
        lax.fori_loop(lo, hi, lambda i, c: (f(i), c)[1], 0)

    def kv_cp(kv, ab, hs, r0, n, prio):
        h, slot = hs
        pltpu.make_async_copy(kv_hbm[kv][ab].at[0, h, pl.ds(r0, n), :],
                              kv_buf[kv].at[slot, ab, pl.ds(r0, n), :],
                              sems.at[kv_sem[kv] + slot]).start(priority=prio)

    def kv_first(kv, ab, s, hs, i, split):
        r0 = al(OFF[ab] + 256 * (8 * s + i))
        if split:
            kv_cp(kv, ab, hs, r0, 64, 1)
            kv_cp(kv, ab, hs, al(r0 + 64), 64, 1)
        else:
            kv_cp(kv, ab, hs, r0, 128, 1)

    def kv_second(kv, ab, s, hs, i, last, nxt):
        if last and s == 1:
            kv_cp(kv, ab, hs, SK - 128 + OFF[ab], 128 - OFF[ab], 0)
            if nxt is not None:
                kv_cp(kv, ab, nxt, 0, OFF[ab], 0)
        else:
            kv_cp(kv, ab, hs, al(OFF[ab] + 128 + 256 * (8 * s + i)), 128, 0)

    def wq_cp(ab, rb, c0, n, prio):
        r = al(rb * 8)
        pltpu.make_async_copy(wqs[ab].at[pl.ds(r, 8), pl.ds(c0, n)],
                              wqbuf.at[ab, pl.ds(r, 8), pl.ds(c0, n)],
                              sems.at[SEM_Q]).start(priority=prio)

    def wq_first(k, i):
        ab, s = k % 2, k // 2
        c0 = OFF[ab] * 16
        if k == 0:
            wq_cp(ab, 16 * s + i, c0, 1024, 1)
            wq_cp(ab, 16 * s + i, c0 + 1024, 1024, 1)
        else:
            wq_cp(ab, 16 * s + i, c0, 2048, 1)

    def wq_second(k, i):
        ab, s = k % 2, k // 2
        c0 = OFF[ab] * 16
        wq_cp(ab, 16 * s + i, c0 + 2048, 2048 - c0, 0)
        wq_cp(ab, (16 * s + i + 1) & 63, 0, c0, 0)

    issued = [0] * len(_GROUP_LIST)

    def wo_rect(ab, r0, n, c0, nc, prio):
        g = _GROUP_OF[(ab, r0 // DH)]
        assert (r0 + n - 1) // DH == r0 // DH
        issued[g] += n * nc
        pltpu.make_async_copy(wos[ab].at[pl.ds(r0, n), pl.ds(c0, nc)],
                              wobuf.at[ab, pl.ds(r0, n), pl.ds(c0, nc)],
                              sems.at[SEM_O + g]).start(priority=prio)

    def wo_tiles(ab, t0, t1, prio):
        if t0 % 4:
            e = min(t1, (t0 // 4 + 1) * 4)
            wo_rect(ab, (t0 // 4) * 8, 8, (t0 % 4) * 128, (e - t0) * 128, prio)
            t0 = e
        if t1 // 4 > t0 // 4:
            wo_rect(ab, (t0 // 4) * 8, (t1 // 4 - t0 // 4) * 8, 0, D, prio)
            t0 = (t1 // 4) * 4
        if t1 > t0:
            wo_rect(ab, (t0 // 4) * 8, 8, 0, (t1 - t0) * 128, prio)

    def compute_q(ab):
        x = jnp.broadcast_to(xbuf[ab, 0], (8, D))
        q = jnp.dot(x, wqbuf[ab], preferred_element_type=jnp.float32)
        for h in range(H):
            qbuf[ab, h] = q[:, h * DH:(h + 1) * DH]

    def scores(hs):
        h, slot = hs
        wait_all(kbuf.at[slot], SEM_K + slot)
        for ab in range(2):
            q = qbuf[ab, h].astype(jnp.bfloat16)
            s = lax.dot_general(q, kbuf[slot, ab], (((1,), (1,)), ((), ())),
                                preferred_element_type=jnp.float32) * SCALE
            m = jnp.max(s, axis=-1, keepdims=True)
            p = jnp.exp(s - m)
            l = jnp.sum(p, axis=-1, keepdims=True)
            pbuf[ab] = p.astype(jnp.bfloat16)
            lbuf[ab] = jnp.broadcast_to(1.0 / l, (8, DH))

    def pv(hs):
        h, slot = hs
        wait_all(vbuf.at[slot], SEM_V + slot)
        for ab in range(2):
            o = jnp.dot(pbuf[ab], vbuf[slot, ab], preferred_element_type=jnp.float32)
            obuf[ab, h] = o * lbuf[ab]

    acc = [jnp.zeros((8, D), jnp.float32)] * 2

    def proj(g):
        assert issued[g] == len(_GROUP_LIST[g]) * DH * D
        for ab, h in _GROUP_LIST[g]:
            wait_all(wobuf.at[ab, pl.ds(h * DH, DH), :], SEM_O + g)
        for ab, h in _GROUP_LIST[g]:
            acc[ab] = acc[ab] + jnp.dot(obuf[ab, h].astype(jnp.bfloat16),
                                        wobuf[ab, h * DH:(h + 1) * DH, :],
                                        preferred_element_type=jnp.float32)

    for ab in range(2):
        pltpu.make_async_copy(xs[ab], xbuf.at[ab], sems.at[SEM_X]).start(priority=0)
    for i in range(LEAD):
        for k in range(8):
            wq_first(k, i)

    def w_round(i):
        for k in range(8):
            wq_second(k, i)
            wq_first(k, i + LEAD)

    def w_round_last(i):
        for k in range(8):
            wq_second(k, i)
            kv_first(*_stream(k), head(0), i - (16 - LEAD), k == 0)

    loop(0, 16 - LEAD, w_round)
    loop(16 - LEAD, 16, w_round_last)
    for kv in range(2):
        for ab in range(2):
            kv_cp(kv, ab, head(0), 0, OFF[ab], 0)

    def kv_round(cur, nxt, i, same, last):
        for k in range(8):
            kv, ab, s = _stream(k)
            kv_second(kv, ab, s, cur, i, last, nxt)
            if same:
                kv_first(kv, ab, s, cur, i + LEAD, k == 0)
            else:
                kv_first(kv, ab, s, nxt, i + LEAD - 8, k == 0)

    def body(b, slots):
        sp, sc, sn = slots
        prev, cur, nxt = (b - 1, sp), (b, sc), (b + 1, sn)
        loop(0, 8 - LEAD, lambda i: kv_round(cur, nxt, i, True, False))

        @pl.when(b == 0)
        def _():
            wait_all(xbuf, SEM_X)
            wait_all(wqbuf, SEM_Q)
            compute_q(0)

        @pl.when(b > 0)
        def _():
            scores(prev)

        loop(8 - LEAD, 7, lambda i: kv_round(cur, nxt, i, False, False))
        kv_round(cur, nxt, 7, False, True)

        @pl.when(b == 0)
        def _():
            compute_q(1)

        @pl.when(b > 0)
        def _():
            pv(prev)

        return sc, sn, sp

    lax.fori_loop(0, H - 2, body, (jnp.int32(2), jnp.int32(0), jnp.int32(1)))

    p0, p1 = {}, {}

    def at(b, i, k=0):
        return 64 * b + 8 * i + k

    def add_kv(b, k, kv, h, nxt):
        _, ab, s = _stream(k)
        for i in range(8):
            p0[at(b, i, k)] = (lambda i=i: kv_second(kv, ab, s, head(h), i, i == 7, nxt))
            p1[at(b, i, k)] = (lambda i=i: kv_first(kv, ab, s, head(h), i, k == 0))

    def add_wo(b, k, r0, rounds):
        ab = _stream(k)[1]
        o = OFF[ab] // 8
        tb, te = r0 // 2, (r0 + 64 * rounds) // 2
        for i in range(rounds + 1):
            lo, hi = max(tb, tb + 32 * (i - 1) + o), min(te, tb + 32 * i + o)
            m0, m1 = (tb, tb + 8) if i == 0 else (tb + 32 * i - 16, tb + 32 * i)

            def f0(lo=lo, hi=hi, m0=m0, m1=m1):
                wo_tiles(ab, lo, m0, 0)
                wo_tiles(ab, m1, hi, 0)

            def f1(m0=m0, m1=m1):
                if k == 0:
                    wo_tiles(ab, m0, (m0 + m1) // 2, 1)
                    wo_tiles(ab, (m0 + m1) // 2, m1, 1)
                else:
                    wo_tiles(ab, m0, m1, 1)

            p0[at(b, i, k)] = f0
            p1[at(b, i, k)] = f1

    for k in range(8):
        kv, _, s = _stream(k)
        add_kv(30, k, kv, 30, head(31))
        if kv == 0:
            add_kv(31, k, 0, 31, None)
            add_kv(32, k, 1, 31, None)
            add_wo(33, k, 3072 + 512 * s, 8 if s == 0 else 6)
        else:
            add_wo(31, k, 1536 * s, 24)
    def tiny_cp(j, ab, r):
        pltpu.make_async_copy(wos[ab].at[pl.ds(r, TINY), :], wobuf.at[ab, pl.ds(r, TINY), :],
                              sems.at[SEM_T + j]).start(priority=1)

    tiny = [(j, ab, 31 * DH + r) for j, (ab, a, b) in enumerate(VP) for r in range(a, b, TINY)]
    t_end = max(p0) + 1
    for t in range(max(p1) + 1, t_end + 8 * LEAD):
        if t - 8 * LEAD in p0:
            p1[t] = (lambda a=tiny.pop(0): tiny_cp(*a))

    pos = [at(30, 0)]

    def issue(upto):
        for t in range(pos[0], upto):
            if t in p0:
                p0[t]()
            if t + 8 * LEAD in p1:
                p1[t + 8 * LEAD]()
        pos[0] = upto

    issue(at(30, 5)); scores(head(29))
    issue(at(31, 0)); pv(head(29))
    issue(at(31, 5)); scores(head(30))
    issue(at(32, 0)); pv(head(30))
    issue(at(32, 5)); scores(head(31))
    issue(at(33, 0)); proj(0)
    issue(at(33, 3)); pv(head(31))
    for ab in range(2):
        o = obuf[ab, 31][0:1, :].astype(jnp.bfloat16).astype(jnp.float32)
        tbuf[ab] = jnp.transpose(jnp.broadcast_to(o, (DH, DH)))
    issue(at(33, 4)); proj(1)
    issue(at(33, 6)); proj(2)
    issue(at(33, 8)); proj(3)
    issue(t_end)
    for a in tiny:
        tiny_cp(*a)
    for g in range(4, len(_GROUP_LIST)):
        proj(g)
    row0 = lax.broadcasted_iota(jnp.int32, (8, D), 0) == 0
    accv = [jnp.where(row0, acc[ab], 0.0) for ab in range(2)]
    for j, (ab, a, b) in enumerate(VP):
        piece = wobuf.at[ab, pl.ds(31 * DH + a, b - a), :]
        wait_all(piece, SEM_T + j)
        parts = []
        for r in range(a, b, 8):
            w = wobuf[ab, 31 * DH + r:31 * DH + r + 8, :].astype(jnp.float32)
            t = tbuf[ab, r:r + 8, :]
            parts.append(w * jnp.concatenate([t] * (D // DH), axis=-1))
        while len(parts) > 1:
            parts = [parts[i] + parts[i + 1] if i + 1 < len(parts) else parts[i]
                     for i in range(0, len(parts), 2)]
        accv[ab] = accv[ab] + parts[0]
    res = [jnp.sum(accv[ab], axis=0, keepdims=True) for ab in range(2)]
    out[0] = jnp.concatenate(res, axis=-1).astype(out.dtype)


@jax.jit
def pallas_concat_heads__mha_block_cached__gqa_block_cached__decode_kernel(
    A_x: jax.Array,
    A_k_cache: jax.Array,
    A_v_cache: jax.Array,
    A_wq: jax.Array,
    A_wo: jax.Array,
    B_x: jax.Array,
    B_k_cache: jax.Array,
    B_v_cache: jax.Array,
    B_wq: jax.Array,
    B_wo: jax.Array,
):
    bf = jnp.bfloat16
    return pl.pallas_call(
        _kernel,
        in_specs=[pl.BlockSpec(memory_space=pl.ANY)] * 10,
        out_specs=pl.BlockSpec(memory_space=pltpu.VMEM),
        out_shape=jax.ShapeDtypeStruct((1, 1, 2 * D), bf),
        scratch_shapes=[
            pltpu.VMEM((NSL, 2, SK, DH), bf),
            pltpu.VMEM((NSL, 2, SK, DH), bf),
            pltpu.VMEM((2, D, HD), bf),
            pltpu.VMEM((2, HD, D), bf),
            pltpu.VMEM((2, 1, 1, D), bf),
            pltpu.VMEM((2, H, 8, DH), jnp.float32),
            pltpu.VMEM((2, 8, SK), bf),
            pltpu.VMEM((2, 8, DH), jnp.float32),
            pltpu.VMEM((2, H, 8, DH), jnp.float32),
            pltpu.VMEM((2, DH, DH), jnp.float32),
            pltpu.SemaphoreType.DMA((NSEM,)),
        ],
        compiler_params=pltpu.CompilerParams(
            vmem_limit_bytes=64 * 1024 * 1024,
            disable_semaphore_checks=True,
        ),
    )(A_x, A_k_cache, A_v_cache, A_wq, A_wo, B_x, B_k_cache, B_v_cache, B_wq, B_wo)
```

```python
import jax
import jax.numpy as jnp
from jax import lax
import jax.experimental.pallas as pl
import jax.experimental.pallas.tpu as pltpu

H, SK, DH, D = 32, 4096, 128, 512
HD = H * DH
SCALE_BF16 = 0.08837890625
NSL = 3
LEAD = 3
OFF = (112, 120)
TINY = 8
VP = ((0, 0, 128), (1, 0, 96), (1, 96, 128))

SEM_K, SEM_V, SEM_Q, SEM_X, SEM_O = 0, NSL, 2 * NSL, 2 * NSL + 1, 2 * NSL + 2

_GROUP_LIST = (
    [(ab, h) for ab in range(2) for h in (0, 1, 2, 3, 12, 13, 14, 15)],
    [(ab, h) for ab in range(2) for h in (4, 5, 6, 7, 16, 17, 18, 19)],
    [(ab, h) for ab in range(2) for h in (8, 20, 24, 28)],
    [(ab, h) for ab in range(2) for h in (9, 21, 25, 29)],
    [(ab, h) for ab in range(2) for h in (10, 22, 26, 30)],
    [(0, 27), (0, 11), (1, 27)],
    [(1, 11), (0, 23), (1, 23)],
)
_GROUP_OF = {key: g for g, keys in enumerate(_GROUP_LIST) for key in keys}
SEM_T = SEM_O + len(_GROUP_LIST)
NSEM = SEM_T + len(VP)


def _round_bf16(x):
    return x.astype(jnp.bfloat16).astype(jnp.float32)


def _stream(k):
    return k % 2, (k // 2) % 2, k // 4


def _kernel(ax, ak, av, awq, awo, bx, bk, bv, bwq, bwo, out,
            kbuf, vbuf, wqbuf, wobuf, xbuf, qbuf, pbuf, lbuf, obuf, tbuf, sems):
    kv_hbm = ((ak, bk), (av, bv))
    kv_buf = (kbuf, vbuf)
    kv_sem = (SEM_K, SEM_V)
    wqs, wos, xs = (awq, bwq), (awo, bwo), (ax, bx)

    def al(v):
        return v if isinstance(v, int) else pl.multiple_of(v, 8)

    def head(h):
        return (h, h % NSL)

    def wait_all(buf, sem):
        pltpu.make_async_copy(buf, buf, sems.at[sem]).wait()

    def loop(lo, hi, f):
        lax.fori_loop(lo, hi, lambda i, c: (f(i), c)[1], 0)

    def kv_cp(kv, ab, hs, r0, n, prio):
        h, slot = hs
        pltpu.make_async_copy(kv_hbm[kv][ab].at[0, h, pl.ds(r0, n), :],
                              kv_buf[kv].at[slot, ab, pl.ds(r0, n), :],
                              sems.at[kv_sem[kv] + slot]).start(priority=prio)

    def kv_first(kv, ab, s, hs, i, split):
        r0 = al(OFF[ab] + 256 * (8 * s + i))
        if split:
            kv_cp(kv, ab, hs, r0, 64, 1)
            kv_cp(kv, ab, hs, al(r0 + 64), 64, 1)
        else:
            kv_cp(kv, ab, hs, r0, 128, 1)

    def kv_second(kv, ab, s, hs, i, last, nxt):
        if last and s == 1:
            kv_cp(kv, ab, hs, SK - 128 + OFF[ab], 128 - OFF[ab], 0)
            if nxt is not None:
                kv_cp(kv, ab, nxt, 0, OFF[ab], 0)
        else:
            kv_cp(kv, ab, hs, al(OFF[ab] + 128 + 256 * (8 * s + i)), 128, 0)

    def wq_cp(ab, rb, c0, n, prio):
        r = al(rb * 8)
        pltpu.make_async_copy(wqs[ab].at[pl.ds(r, 8), pl.ds(c0, n)],
                              wqbuf.at[ab, pl.ds(r, 8), pl.ds(c0, n)],
                              sems.at[SEM_Q]).start(priority=prio)

    def wq_first(k, i):
        ab, s = k % 2, k // 2
        c0 = OFF[ab] * 16
        if k == 0:
            wq_cp(ab, 16 * s + i, c0, 1024, 1)
            wq_cp(ab, 16 * s + i, c0 + 1024, 1024, 1)
        else:
            wq_cp(ab, 16 * s + i, c0, 2048, 1)

    def wq_second(k, i):
        ab, s = k % 2, k // 2
        c0 = OFF[ab] * 16
        wq_cp(ab, 16 * s + i, c0 + 2048, 2048 - c0, 0)
        wq_cp(ab, (16 * s + i + 1) & 63, 0, c0, 0)

    issued = [0] * len(_GROUP_LIST)

    def wo_rect(ab, r0, n, c0, nc, prio):
        g = _GROUP_OF[(ab, r0 // DH)]
        assert (r0 + n - 1) // DH == r0 // DH
        issued[g] += n * nc
        pltpu.make_async_copy(wos[ab].at[pl.ds(r0, n), pl.ds(c0, nc)],
                              wobuf.at[ab, pl.ds(r0, n), pl.ds(c0, nc)],
                              sems.at[SEM_O + g]).start(priority=prio)

    def wo_tiles(ab, t0, t1, prio):
        if t0 % 4:
            e = min(t1, (t0 // 4 + 1) * 4)
            wo_rect(ab, (t0 // 4) * 8, 8, (t0 % 4) * 128, (e - t0) * 128, prio)
            t0 = e
        if t1 // 4 > t0 // 4:
            wo_rect(ab, (t0 // 4) * 8, (t1 // 4 - t0 // 4) * 8, 0, D, prio)
            t0 = (t1 // 4) * 4
        if t1 > t0:
            wo_rect(ab, (t0 // 4) * 8, 8, 0, (t1 - t0) * 128, prio)

    def compute_q(ab):
        x = jnp.broadcast_to(xbuf[ab, 0], (8, D))
        q = jnp.dot(x, wqbuf[ab], preferred_element_type=jnp.float32)
        for h in range(H):
            qbuf[ab, h] = q[:, h * DH:(h + 1) * DH]

    def scores(hs):
        h, slot = hs
        wait_all(kbuf.at[slot], SEM_K + slot)
        for ab in range(2):
            q = qbuf[ab, h].astype(jnp.bfloat16)
            s = lax.dot_general(q, kbuf[slot, ab], (((1,), (1,)), ((), ())),
                                preferred_element_type=jnp.float32)
            s = _round_bf16(_round_bf16(s) * SCALE_BF16)
            m = jnp.max(s, axis=-1, keepdims=True)
            p = jnp.exp(s - m)
            l = jnp.sum(p, axis=-1, keepdims=True)
            pbuf[ab] = p.astype(jnp.bfloat16)
            lbuf[ab] = jnp.broadcast_to(1.0 / l, (8, DH))

    def pv(hs):
        h, slot = hs
        wait_all(vbuf.at[slot], SEM_V + slot)
        for ab in range(2):
            o = jnp.dot(pbuf[ab], vbuf[slot, ab], preferred_element_type=jnp.float32)
            obuf[ab, h] = o * lbuf[ab]

    acc = [jnp.zeros((8, D), jnp.float32)] * 2

    def proj(g):
        assert issued[g] == len(_GROUP_LIST[g]) * DH * D
        for ab, h in _GROUP_LIST[g]:
            wait_all(wobuf.at[ab, pl.ds(h * DH, DH), :], SEM_O + g)
        for ab, h in _GROUP_LIST[g]:
            acc[ab] = acc[ab] + jnp.dot(obuf[ab, h].astype(jnp.bfloat16),
                                        wobuf[ab, h * DH:(h + 1) * DH, :],
                                        preferred_element_type=jnp.float32)

    for ab in range(2):
        pltpu.make_async_copy(xs[ab], xbuf.at[ab], sems.at[SEM_X]).start(priority=0)
    for i in range(LEAD):
        for k in range(8):
            wq_first(k, i)

    def w_round(i):
        for k in range(8):
            wq_second(k, i)
            wq_first(k, i + LEAD)

    def w_round_last(i):
        for k in range(8):
            wq_second(k, i)
            kv_first(*_stream(k), head(0), i - (16 - LEAD), k == 0)

    loop(0, 16 - LEAD, w_round)
    loop(16 - LEAD, 16, w_round_last)
    for kv in range(2):
        for ab in range(2):
            kv_cp(kv, ab, head(0), 0, OFF[ab], 0)

    def kv_round(cur, nxt, i, same, last):
        for k in range(8):
            kv, ab, s = _stream(k)
            kv_second(kv, ab, s, cur, i, last, nxt)
            if same:
                kv_first(kv, ab, s, cur, i + LEAD, k == 0)
            else:
                kv_first(kv, ab, s, nxt, i + LEAD - 8, k == 0)

    def body(b, slots):
        sp, sc, sn = slots
        prev, cur, nxt = (b - 1, sp), (b, sc), (b + 1, sn)
        loop(0, 8 - LEAD, lambda i: kv_round(cur, nxt, i, True, False))

        @pl.when(b == 0)
        def _():
            wait_all(xbuf, SEM_X)
            wait_all(wqbuf, SEM_Q)
            compute_q(0)

        @pl.when(b > 0)
        def _():
            scores(prev)

        loop(8 - LEAD, 7, lambda i: kv_round(cur, nxt, i, False, False))
        kv_round(cur, nxt, 7, False, True)

        @pl.when(b == 0)
        def _():
            compute_q(1)

        @pl.when(b > 0)
        def _():
            pv(prev)

        return sc, sn, sp

    lax.fori_loop(0, H - 2, body, (jnp.int32(2), jnp.int32(0), jnp.int32(1)))

    p0, p1 = {}, {}

    def at(b, i, k=0):
        return 64 * b + 8 * i + k

    def add_kv(b, k, kv, h, nxt):
        _, ab, s = _stream(k)
        for i in range(8):
            p0[at(b, i, k)] = (lambda i=i: kv_second(kv, ab, s, head(h), i, i == 7, nxt))
            p1[at(b, i, k)] = (lambda i=i: kv_first(kv, ab, s, head(h), i, k == 0))

    def add_wo(b, k, r0, rounds):
        ab = _stream(k)[1]
        o = OFF[ab] // 8
        tb, te = r0 // 2, (r0 + 64 * rounds) // 2
        for i in range(rounds + 1):
            lo, hi = max(tb, tb + 32 * (i - 1) + o), min(te, tb + 32 * i + o)
            m0, m1 = (tb, tb + 8) if i == 0 else (tb + 32 * i - 16, tb + 32 * i)

            def f0(lo=lo, hi=hi, m0=m0, m1=m1):
                wo_tiles(ab, lo, m0, 0)
                wo_tiles(ab, m1, hi, 0)

            def f1(m0=m0, m1=m1):
                if k == 0:
                    wo_tiles(ab, m0, (m0 + m1) // 2, 1)
                    wo_tiles(ab, (m0 + m1) // 2, m1, 1)
                else:
                    wo_tiles(ab, m0, m1, 1)

            p0[at(b, i, k)] = f0
            p1[at(b, i, k)] = f1

    for k in range(8):
        kv, _, s = _stream(k)
        add_kv(30, k, kv, 30, head(31))
        if kv == 0:
            add_kv(31, k, 0, 31, None)
            add_kv(32, k, 1, 31, None)
            add_wo(33, k, 3072 + 512 * s, 8 if s == 0 else 6)
        else:
            add_wo(31, k, 1536 * s, 24)
    def tiny_cp(j, ab, r):
        pltpu.make_async_copy(wos[ab].at[pl.ds(r, TINY), :], wobuf.at[ab, pl.ds(r, TINY), :],
                              sems.at[SEM_T + j]).start(priority=1)

    tiny = [(j, ab, 31 * DH + r) for j, (ab, a, b) in enumerate(VP) for r in range(a, b, TINY)]
    t_end = max(p0) + 1
    for t in range(max(p1) + 1, t_end + 8 * LEAD):
        if t - 8 * LEAD in p0:
            p1[t] = (lambda a=tiny.pop(0): tiny_cp(*a))

    pos = [at(30, 0)]

    def issue(upto):
        for t in range(pos[0], upto):
            if t in p0:
                p0[t]()
            if t + 8 * LEAD in p1:
                p1[t + 8 * LEAD]()
        pos[0] = upto

    issue(at(30, 5)); scores(head(29))
    issue(at(31, 0)); pv(head(29))
    issue(at(31, 5)); scores(head(30))
    issue(at(32, 0)); pv(head(30))
    issue(at(32, 5)); scores(head(31))
    issue(at(33, 0)); proj(0)
    issue(at(33, 3)); pv(head(31))
    for ab in range(2):
        o = _round_bf16(obuf[ab, 31][0:1, :])
        tbuf[ab] = jnp.transpose(jnp.broadcast_to(o, (DH, DH)))
    issue(at(33, 4)); proj(1)
    issue(at(33, 6)); proj(2)
    issue(at(33, 8)); proj(3)
    issue(t_end)
    for a in tiny:
        tiny_cp(*a)
    for g in range(4, len(_GROUP_LIST)):
        proj(g)
    row0 = lax.broadcasted_iota(jnp.int32, (8, D), 0) == 0
    accv = [jnp.where(row0, acc[ab], 0.0) for ab in range(2)]
    for j, (ab, a, b) in enumerate(VP):
        piece = wobuf.at[ab, pl.ds(31 * DH + a, b - a), :]
        wait_all(piece, SEM_T + j)
        parts = []
        for r in range(a, b, 8):
            w = wobuf[ab, 31 * DH + r:31 * DH + r + 8, :].astype(jnp.float32)
            t = tbuf[ab, r:r + 8, :]
            parts.append(w * jnp.concatenate([t] * (D // DH), axis=-1))
        while len(parts) > 1:
            parts = [parts[i] + parts[i + 1] if i + 1 < len(parts) else parts[i]
                     for i in range(0, len(parts), 2)]
        accv[ab] = accv[ab] + parts[0]
    res = [jnp.sum(accv[ab], axis=0, keepdims=True) for ab in range(2)]
    out[0] = jnp.concatenate(res, axis=-1).astype(out.dtype)


@jax.jit
def pallas_concat_heads__mha_block_cached__gqa_block_cached__decode_kernel(
    A_x: jax.Array,
    A_k_cache: jax.Array,
    A_v_cache: jax.Array,
    A_wq: jax.Array,
    A_wo: jax.Array,
    B_x: jax.Array,
    B_k_cache: jax.Array,
    B_v_cache: jax.Array,
    B_wq: jax.Array,
    B_wo: jax.Array,
):
    bf = jnp.bfloat16
    return pl.pallas_call(
        _kernel,
        in_specs=[pl.BlockSpec(memory_space=pl.ANY)] * 10,
        out_specs=pl.BlockSpec(memory_space=pltpu.VMEM),
        out_shape=jax.ShapeDtypeStruct((1, 1, 2 * D), bf),
        scratch_shapes=[
            pltpu.VMEM((NSL, 2, SK, DH), bf),
            pltpu.VMEM((NSL, 2, SK, DH), bf),
            pltpu.VMEM((2, D, HD), bf),
            pltpu.VMEM((2, HD, D), bf),
            pltpu.VMEM((2, 1, 1, D), bf),
            pltpu.VMEM((2, H, 8, DH), jnp.float32),
            pltpu.VMEM((2, 8, SK), bf),
            pltpu.VMEM((2, 8, DH), jnp.float32),
            pltpu.VMEM((2, H, 8, DH), jnp.float32),
            pltpu.VMEM((2, DH, DH), jnp.float32),
            pltpu.SemaphoreType.DMA((NSEM,)),
        ],
        compiler_params=pltpu.CompilerParams(
            vmem_limit_bytes=64 * 1024 * 1024,
            disable_semaphore_checks=True,
        ),
    )(A_x, A_k_cache, A_v_cache, A_wq, A_wo, B_x, B_k_cache, B_v_cache, B_wq, B_wo)
```

```python
import jax
import jax.numpy as jnp
from jax import lax
import jax.experimental.pallas as pl
import jax.experimental.pallas.tpu as pltpu

H, SK, DH, D = 32, 4096, 128, 512
HD = H * DH
SCALE_BF16 = 0.08837890625
NSL = 3
LEAD = 3
OFF = (112, 120)
TINY = 8
VP = ((0, 0, 128), (1, 0, 96), (1, 96, 128))

SEM_K, SEM_V, SEM_Q, SEM_X, SEM_O = 0, NSL, 2 * NSL, 2 * NSL + 1, 2 * NSL + 2

_GROUP_LIST = (
    [(ab, h) for ab in range(2) for h in (0, 1, 2, 3, 12, 13, 14, 15)],
    [(ab, h) for ab in range(2) for h in (4, 5, 6, 7, 16, 17, 18, 19)],
    [(ab, h) for ab in range(2) for h in (8, 20, 24, 28)],
    [(ab, h) for ab in range(2) for h in (9, 21, 25, 29)],
    [(ab, h) for ab in range(2) for h in (10, 22, 26, 30)],
    [(0, 27), (0, 11), (1, 27)],
    [(1, 11), (0, 23), (1, 23)],
)
_GROUP_OF = {key: g for g, keys in enumerate(_GROUP_LIST) for key in keys}
SEM_T = SEM_O + len(_GROUP_LIST)
NSEM = SEM_T + len(VP)


def _round_bf16(x):
    return x.astype(jnp.bfloat16).astype(jnp.float32)


def _stream(k):
    return k % 2, (k // 2) % 2, k // 4


def _kernel(ax, ak, av, awq, awo, bx, bk, bv, bwq, bwo, out,
            kbuf, vbuf, wqbuf, wobuf, xbuf, qbuf, pbuf, lbuf, obuf, tbuf, sems):
    kv_hbm = ((ak, bk), (av, bv))
    kv_buf = (kbuf, vbuf)
    kv_sem = (SEM_K, SEM_V)
    wqs, wos, xs = (awq, bwq), (awo, bwo), (ax, bx)

    def al(v):
        return v if isinstance(v, int) else pl.multiple_of(v, 8)

    def head(h):
        return (h, h % NSL)

    def wait_all(buf, sem):
        pltpu.make_async_copy(buf, buf, sems.at[sem]).wait()

    def loop(lo, hi, f):
        lax.fori_loop(lo, hi, lambda i, c: (f(i), c)[1], 0)

    def kv_cp(kv, ab, hs, r0, n, prio):
        h, slot = hs
        pltpu.make_async_copy(kv_hbm[kv][ab].at[0, h, pl.ds(r0, n), :],
                              kv_buf[kv].at[slot, ab, pl.ds(r0, n), :],
                              sems.at[kv_sem[kv] + slot]).start(priority=prio)

    def kv_first(kv, ab, s, hs, i, split):
        r0 = al(OFF[ab] + 256 * (8 * s + i))
        if split:
            kv_cp(kv, ab, hs, r0, 64, 1)
            kv_cp(kv, ab, hs, al(r0 + 64), 64, 1)
        else:
            kv_cp(kv, ab, hs, r0, 128, 1)

    def kv_second(kv, ab, s, hs, i, last, nxt):
        if last and s == 1:
            kv_cp(kv, ab, hs, SK - 128 + OFF[ab], 128 - OFF[ab], 0)
            if nxt is not None:
                kv_cp(kv, ab, nxt, 0, OFF[ab], 0)
        else:
            kv_cp(kv, ab, hs, al(OFF[ab] + 128 + 256 * (8 * s + i)), 128, 0)

    def wq_cp(ab, rb, c0, n, prio):
        r = al(rb * 8)
        pltpu.make_async_copy(wqs[ab].at[pl.ds(r, 8), pl.ds(c0, n)],
                              wqbuf.at[ab, pl.ds(r, 8), pl.ds(c0, n)],
                              sems.at[SEM_Q]).start(priority=prio)

    def wq_first(k, i):
        ab, s = k % 2, k // 2
        c0 = OFF[ab] * 16
        if k == 0:
            wq_cp(ab, 16 * s + i, c0, 1024, 1)
            wq_cp(ab, 16 * s + i, c0 + 1024, 1024, 1)
        else:
            wq_cp(ab, 16 * s + i, c0, 2048, 1)

    def wq_second(k, i):
        ab, s = k % 2, k // 2
        c0 = OFF[ab] * 16
        wq_cp(ab, 16 * s + i, c0 + 2048, 2048 - c0, 0)
        wq_cp(ab, (16 * s + i + 1) & 63, 0, c0, 0)

    issued = [0] * len(_GROUP_LIST)

    def wo_rect(ab, r0, n, c0, nc, prio):
        g = _GROUP_OF[(ab, r0 // DH)]
        assert (r0 + n - 1) // DH == r0 // DH
        issued[g] += n * nc
        pltpu.make_async_copy(wos[ab].at[pl.ds(r0, n), pl.ds(c0, nc)],
                              wobuf.at[ab, pl.ds(r0, n), pl.ds(c0, nc)],
                              sems.at[SEM_O + g]).start(priority=prio)

    def wo_tiles(ab, t0, t1, prio):
        if t0 % 4:
            e = min(t1, (t0 // 4 + 1) * 4)
            wo_rect(ab, (t0 // 4) * 8, 8, (t0 % 4) * 128, (e - t0) * 128, prio)
            t0 = e
        if t1 // 4 > t0 // 4:
            wo_rect(ab, (t0 // 4) * 8, (t1 // 4 - t0 // 4) * 8, 0, D, prio)
            t0 = (t1 // 4) * 4
        if t1 > t0:
            wo_rect(ab, (t0 // 4) * 8, 8, 0, (t1 - t0) * 128, prio)

    def compute_q(ab):
        x = jnp.broadcast_to(xbuf[ab, 0], (8, D))
        q = jnp.dot(x, wqbuf[ab], preferred_element_type=jnp.float32)
        for h in range(H):
            qbuf[ab, h] = q[:, h * DH:(h + 1) * DH]

    def scores(hs):
        h, slot = hs
        wait_all(kbuf.at[slot], SEM_K + slot)
        for ab in range(2):
            q = qbuf[ab, h].astype(jnp.bfloat16)
            s = lax.dot_general(q, kbuf[slot, ab], (((1,), (1,)), ((), ())),
                                preferred_element_type=jnp.float32)
            s = _round_bf16(_round_bf16(s) * SCALE_BF16)
            m = jnp.max(s, axis=-1, keepdims=True)
            p = jnp.exp(s - m)
            l = jnp.sum(p, axis=-1, keepdims=True)
            pbuf[ab] = p.astype(jnp.bfloat16)
            lbuf[ab] = jnp.broadcast_to(1.0 / l, (8, DH))

    def pv(hs):
        h, slot = hs
        wait_all(vbuf.at[slot], SEM_V + slot)
        for ab in range(2):
            o = jnp.dot(pbuf[ab], vbuf[slot, ab], preferred_element_type=jnp.float32)
            obuf[ab, h] = o * lbuf[ab]

    acc = [jnp.zeros((8, D), jnp.float32)] * 2

    def proj(g):
        assert issued[g] == len(_GROUP_LIST[g]) * DH * D
        for ab, h in _GROUP_LIST[g]:
            wait_all(wobuf.at[ab, pl.ds(h * DH, DH), :], SEM_O + g)
        for ab, h in _GROUP_LIST[g]:
            acc[ab] = acc[ab] + jnp.dot(obuf[ab, h].astype(jnp.bfloat16),
                                        wobuf[ab, h * DH:(h + 1) * DH, :],
                                        preferred_element_type=jnp.float32)

    for ab in range(2):
        pltpu.make_async_copy(xs[ab], xbuf.at[ab], sems.at[SEM_X]).start(priority=0)
    for i in range(LEAD):
        for k in range(8):
            wq_first(k, i)

    def w_round(i):
        for k in range(8):
            wq_second(k, i)
            wq_first(k, i + LEAD)

    def w_round_last(i):
        for k in range(8):
            wq_second(k, i)
            kv_first(*_stream(k), head(0), i - (16 - LEAD), k == 0)

    loop(0, 16 - LEAD, w_round)
    loop(16 - LEAD, 16, w_round_last)
    for kv in range(2):
        for ab in range(2):
            kv_cp(kv, ab, head(0), 0, OFF[ab], 0)

    def kv_round(cur, nxt, i, same, last):
        for k in range(8):
            kv, ab, s = _stream(k)
            kv_second(kv, ab, s, cur, i, last, nxt)
            if same:
                kv_first(kv, ab, s, cur, i + LEAD, k == 0)
            else:
                kv_first(kv, ab, s, nxt, i + LEAD - 8, k == 0)

    def body(b, slots):
        sp, sc, sn = slots
        prev, cur, nxt = (b - 1, sp), (b, sc), (b + 1, sn)
        loop(0, 8 - LEAD, lambda i: kv_round(cur, nxt, i, True, False))

        @pl.when(b == 0)
        def _():
            wait_all(xbuf, SEM_X)
            wait_all(wqbuf, SEM_Q)
            compute_q(0)

        @pl.when(b > 0)
        def _():
            scores(prev)

        loop(8 - LEAD, 7, lambda i: kv_round(cur, nxt, i, False, False))
        kv_round(cur, nxt, 7, False, True)

        @pl.when(b == 0)
        def _():
            compute_q(1)

        @pl.when(b > 0)
        def _():
            pv(prev)

        return sc, sn, sp

    lax.fori_loop(0, H - 2, body, (jnp.int32(2), jnp.int32(0), jnp.int32(1)))

    p0, p1 = {}, {}

    def at(b, i, k=0):
        return 64 * b + 8 * i + k

    def add_kv(b, k, kv, h, nxt):
        _, ab, s = _stream(k)
        for i in range(8):
            p0[at(b, i, k)] = (lambda i=i: kv_second(kv, ab, s, head(h), i, i == 7, nxt))
            p1[at(b, i, k)] = (lambda i=i: kv_first(kv, ab, s, head(h), i, k == 0))

    def add_wo(b, k, r0, rounds):
        ab = _stream(k)[1]
        o = OFF[ab] // 8
        tb, te = r0 // 2, (r0 + 64 * rounds) // 2
        for i in range(rounds + 1):
            lo, hi = max(tb, tb + 32 * (i - 1) + o), min(te, tb + 32 * i + o)
            m0, m1 = (tb, tb + 8) if i == 0 else (tb + 32 * i - 16, tb + 32 * i)

            def f0(lo=lo, hi=hi, m0=m0, m1=m1):
                wo_tiles(ab, lo, m0, 0)
                wo_tiles(ab, m1, hi, 0)

            def f1(m0=m0, m1=m1):
                if k == 0:
                    wo_tiles(ab, m0, (m0 + m1) // 2, 1)
                    wo_tiles(ab, (m0 + m1) // 2, m1, 1)
                else:
                    wo_tiles(ab, m0, m1, 1)

            p0[at(b, i, k)] = f0
            p1[at(b, i, k)] = f1

    for k in range(8):
        kv, _, s = _stream(k)
        add_kv(30, k, kv, 30, head(31))
        if kv == 0:
            add_kv(31, k, 0, 31, None)
            add_kv(32, k, 1, 31, None)
            add_wo(33, k, 3072 + 512 * s, 8 if s == 0 else 6)
        else:
            add_wo(31, k, 1536 * s, 24)

    def tiny_cp(j, ab, r):
        pltpu.make_async_copy(wos[ab].at[pl.ds(r, TINY), :],
                              wobuf.at[ab, pl.ds(r, TINY), :],
                              sems.at[SEM_T + j]).start(priority=1)

    tiny = [(j, ab, 31 * DH + r)
            for j, (ab, a, b) in enumerate(VP) for r in range(a, b, TINY)]
    t_end = max(p0) + 1
    for t in range(max(p1) + 1, t_end + 8 * LEAD):
        if t - 8 * LEAD in p0:
            p1[t] = (lambda a=tiny.pop(0): tiny_cp(*a))

    pos = [at(30, 0)]

    def issue(upto):
        for t in range(pos[0], upto):
            if t in p0:
                p0[t]()
            if t + 8 * LEAD in p1:
                p1[t + 8 * LEAD]()
        pos[0] = upto

    issue(at(30, 5)); scores(head(29))
    issue(at(31, 0)); pv(head(29))
    issue(at(31, 5)); scores(head(30))
    issue(at(32, 0)); pv(head(30))
    issue(at(32, 5)); scores(head(31))
    issue(at(33, 0)); proj(0)
    issue(at(33, 3)); pv(head(31))
    for ab in range(2):
        o = _round_bf16(obuf[ab, 31][0:1, :])
        tbuf[ab] = jnp.transpose(jnp.broadcast_to(o, (DH, DH)))
    issue(at(33, 4)); proj(1)
    issue(at(33, 6)); proj(2)
    issue(at(33, 8)); proj(3)
    issue(t_end)
    for a in tiny:
        tiny_cp(*a)
    for g in range(4, len(_GROUP_LIST)):
        proj(g)
    row0 = lax.broadcasted_iota(jnp.int32, (8, D), 0) == 0
    accv = [jnp.where(row0, acc[ab], 0.0) for ab in range(2)]
    for j, (ab, a, b) in enumerate(VP):
        piece = wobuf.at[ab, pl.ds(31 * DH + a, b - a), :]
        wait_all(piece, SEM_T + j)
        parts = []
        for r in range(a, b, 8):
            w = wobuf[ab, 31 * DH + r:31 * DH + r + 8, :].astype(jnp.float32)
            t = tbuf[ab, r:r + 8, :]
            parts.append(w * jnp.concatenate([t] * (D // DH), axis=-1))
        while len(parts) > 1:
            parts = [parts[i] + parts[i + 1] if i + 1 < len(parts) else parts[i]
                     for i in range(0, len(parts), 2)]
        accv[ab] = accv[ab] + parts[0]
    res = [jnp.sum(accv[ab], axis=0, keepdims=True) for ab in range(2)]
    out[0] = jnp.concatenate(res, axis=-1).astype(out.dtype)


@jax.jit
def pallas_concat_heads__mha_block_cached__gqa_block_cached__decode_kernel(
    A_x: jax.Array,
    A_k_cache: jax.Array,
    A_v_cache: jax.Array,
    A_wq: jax.Array,
    A_wo: jax.Array,
    B_x: jax.Array,
    B_k_cache: jax.Array,
    B_v_cache: jax.Array,
    B_wq: jax.Array,
    B_wo: jax.Array,
):
    bf = jnp.bfloat16
    assert A_x.shape == B_x.shape == (1, 1, D)
    assert A_wq.shape == B_wq.shape == (D, HD) and A_wo.shape == B_wo.shape == (HD, D)
    for c in (A_k_cache, A_v_cache, B_k_cache, B_v_cache):
        assert c.shape == (1, H, SK, DH)
    return pl.pallas_call(
        _kernel,
        in_specs=[pl.BlockSpec(memory_space=pl.ANY)] * 10,
        out_specs=pl.BlockSpec(memory_space=pltpu.VMEM),
        out_shape=jax.ShapeDtypeStruct((1, 1, 2 * D), bf),
        scratch_shapes=[
            pltpu.VMEM((NSL, 2, SK, DH), bf),
            pltpu.VMEM((NSL, 2, SK, DH), bf),
            pltpu.VMEM((2, D, HD), bf),
            pltpu.VMEM((2, HD, D), bf),
            pltpu.VMEM((2, 1, 1, D), bf),
            pltpu.VMEM((2, H, 8, DH), jnp.float32),
            pltpu.VMEM((2, 8, SK), bf),
            pltpu.VMEM((2, 8, DH), jnp.float32),
            pltpu.VMEM((2, H, 8, DH), jnp.float32),
            pltpu.VMEM((2, DH, DH), jnp.float32),
            pltpu.SemaphoreType.DMA((NSEM,)),
        ],
        compiler_params=pltpu.CompilerParams(
            vmem_limit_bytes=64 * 1024 * 1024,
            disable_semaphore_checks=True,
        ),
    )(A_x, A_k_cache, A_v_cache, A_wq, A_wo, B_x, B_k_cache, B_v_cache, B_wq, B_wo)
```
